```python
import os as _os
_os.environ.setdefault("JAX_PLATFORMS", "cpu")
import jax
import jax.numpy as jnp

def _softmax(x, axis=-1):
    return jax.nn.softmax(x, axis=axis)
def _gelu(x):
    return jax.nn.gelu(x, approximate=True)
def _silu(x):
    return jax.nn.silu(x)
def _sigmoid(x):
    return jax.nn.sigmoid(x)
def _layernorm(x, axis=-1, eps=1e-5):
    m = jnp.mean(x, axis=axis, keepdims=True)
    v = jnp.var(x, axis=axis, keepdims=True)
    return (x - m) / jnp.sqrt(v + eps)
def _scatter_add(tgt, idx, src, axis=0):
    return tgt.at[idx].add(src)
def _segment_sum(src, seg, n):
    return jax.ops.segment_sum(src, seg, n)
class _Rng:
    def __init__(self, key):
        self._k = key
    def _next(self):
        self._k, sub = jax.random.split(self._k)
        return sub
    def normal(self, shape):
        return jax.random.normal(self._next(), shape, dtype=jnp.bfloat16)
    def randint(self, lo, hi, shape):
        return jax.random.randint(self._next(), shape, lo, hi, dtype=jnp.int32)
    def uniform(self, shape, lo=0.0, hi=1.0):
        return jax.random.uniform(self._next(), shape, jnp.bfloat16, lo, hi)
    def permutation(self, n):
        return jax.random.permutation(self._next(), n)


kernel_name = 'interleave_layers__linear_kernel_hedgehog__dense_activation_silu__prompt'

def setup_inputs():
    _rng = _Rng(jax.random.key(int.from_bytes(__import__("os").urandom(4), "little")))
    _w = (lambda a: (lambda t: t.astype(jnp.bfloat16) if jnp.issubdtype(t.dtype, jnp.floating) else t)(jnp.asarray(a)))
    def _A_setup():
        B, S, D, H = 1, 2048, 640, 32
        Dh = D // H
        return {
            "x": _w((lambda *s: _rng.normal(s) * 0.05)(B, S, D)),
            "wqkv": _w((lambda *s: _rng.normal(s) * 0.4)(D, 3 * D)),
            "w_phi": _w((lambda *s: _rng.normal(s) * 0.4)(H, Dh, Dh) * (Dh ** -0.5)),
            "wo": _w((lambda *s: _rng.normal(s) * 0.05)(D, D)),
        }
    _A_in = _A_setup()

    def _B_setup():
        B, S, D, F = 1, 2048, 640, 1728
        return {
            "x": _w((lambda *s: _rng.normal(s) * 0.05)(B, S, D)),
            "w1": _w((lambda *s: _rng.normal(s) * 1.6)(D, F) * (D ** -0.5)),
            "w2": _w((lambda *s: _rng.normal(s) * 1.6)(F, D) * (F ** -0.5)),
        }
    _B_in = _B_setup()

    return {
        "A_x": _A_in["x"],
        "A_wqkv": _A_in["wqkv"],
        "A_w_phi": _A_in["w_phi"],
        "A_wo": _A_in["wo"],
        "B_x": _B_in["x"],
        "B_w1": _B_in["w1"],
        "B_w2": _B_in["w2"],
    }

def reference(A_x, A_wqkv, A_w_phi, A_wo, B_x, B_w1, B_w2):
    def _A_ref(x, wqkv, w_phi, wo):
        B, S, D = x.shape
        H = 32; Dh = D // H
        qkv = (lambda x, *d: x.transpose(*d))((x @ wqkv).reshape(B, S, 3, H, Dh), 2, 0, 3, 1, 4)
        q, k, v = qkv[0], qkv[1], qkv[2]
        pq = jnp.einsum("bhsd,hdf->bhsf", q, w_phi)
        pk = jnp.einsum("bhsd,hdf->bhsf", k, w_phi)
        phi_q = jnp.concatenate([_softmax(pq, axis=-1), _softmax(-pq, axis=-1)], axis=-1)
        phi_k = jnp.concatenate([_softmax(pk, axis=-1), _softmax(-pk, axis=-1)], axis=-1)
        kv = jnp.einsum("bhsf,bhsd->bhfd", phi_k, v)
        z  = jnp.einsum("bhsf->bhf", phi_k)
        num = jnp.einsum("bhqf,bhfd->bhqd", phi_q, kv)
        den = jnp.einsum("bhqf,bhf->bhq", phi_q, z)[..., None] + 1e-6
        o = num / den
        return (lambda x, *d: x.transpose(*d))(o, 0, 2, 1, 3).reshape(B, S, D) @ wo

    def _B_ref(x, w1, w2):
        h = jnp.einsum("bsd,df->bsf", x, w1)
        h = _silu(h)
        out = jnp.einsum("bsf,fd->bsd", h, w2)
        return out

    x = A_x
    x = x + _A_ref(_layernorm(x, axis=-1), A_wqkv, A_w_phi, A_wo)
    x = x + _B_ref(_layernorm(x, axis=-1), B_w1, B_w2)
    x = x + _A_ref(_layernorm(x, axis=-1), A_wqkv, A_w_phi, A_wo)
    x = x + _B_ref(_layernorm(x, axis=-1), B_w1, B_w2)
    return x
```

```python
import functools

import jax
import jax.numpy as jnp
import jax.experimental.pallas as pl
import jax.experimental.pallas.tpu as pltpu

S, D, H, DH, F = 2048, 640, 32, 20, 1728
HP = 24
RQ = H * HP
NCH, HPC = 8, 4
CR = HPC * HP
CV = HPC * DH
EPS_LN = 1e-5
NEG = -1e30


def _layernorm(x):
    m = jnp.mean(x, axis=-1, keepdims=True)
    xc = x - m
    v = jnp.mean(xc * xc, axis=-1, keepdims=True)
    return xc * jax.lax.rsqrt(v + EPS_LN)


def _dot(a, b):
    return jnp.dot(a, b, preferred_element_type=jnp.float32)


def _dg(a, b, ca, cb):
    return jax.lax.dot_general(a, b, (((ca,), (cb,)), ((), ())), preferred_element_type=jnp.float32)


def _kernel(x_ref, wqkv_ref, wpht_ref, wo_ref, w1_ref, w2_ref, o_ref,
            x_vm, wqkt_vm, phiq_st, kvz_acc, *, tp):
    n_tiles = S // tp

    r = jax.lax.broadcasted_iota(jnp.int32, (RQ, D), 0)
    c = jax.lax.broadcasted_iota(jnp.int32, (RQ, D), 1)
    bd_mask = (r // HP) == (c // DH)
    tiled = jnp.concatenate([wpht_ref[...]] * H, axis=1)
    bdt = jnp.where(bd_mask, tiled, jnp.zeros_like(tiled))
    wqkt_vm[0:RQ, :] = _dg(bdt, wqkv_ref[:, 0:D], 1, 1).astype(jnp.bfloat16)
    wqkt_vm[RQ:2 * RQ, :] = _dg(bdt, wqkv_ref[:, D:2 * D], 1, 1).astype(jnp.bfloat16)
    x_vm[...] = x_ref[...].astype(jnp.float32)

    rowt = jax.lax.broadcasted_iota(jnp.int32, (2 * RQ, tp), 0)
    valid = (rowt % HP) < DH
    ones_pad = jnp.ones((128 - CV, tp), jnp.bfloat16)
    rr = jax.lax.broadcasted_iota(jnp.int32, (2 * CR, CV), 0)
    cc = jax.lax.broadcasted_iota(jnp.int32, (2 * CR, CV), 1)
    bdmask2 = ((rr % CR) // HP) == (cc // DH)

    def softmax_branches(pT):
        outs = []
        for sgn in (1.0, -1.0):
            z = jnp.where(valid, sgn * pT, NEG).reshape(2 * H, HP, tp)
            m = jnp.max(z, axis=1, keepdims=True)
            e = jnp.exp(z - m)
            sm = jnp.sum(e, axis=1, keepdims=True)
            p = (e * (1.0 / sm)).reshape(2 * RQ, tp)
            outs.append(jnp.where(valid, p, 0.0).astype(jnp.bfloat16))
        return outs

    def layer_a():
        kvz_acc[...] = jnp.zeros_like(kvz_acc)
        wqkt = wqkt_vm[...]
        for t in range(n_tiles):
            xt = x_vm[t * tp:(t + 1) * tp, :]
            l = _layernorm(xt).astype(jnp.bfloat16)
            pT = _dg(wqkt, l, 1, 1)
            vT = _dg(wqkv_ref[:, 2 * D:3 * D], l, 0, 1).astype(jnp.bfloat16)
            phi_pos, phi_neg = softmax_branches(pT)
            phiq_st[0:RQ, t * tp:(t + 1) * tp] = phi_pos[0:RQ]
            phiq_st[RQ:2 * RQ, t * tp:(t + 1) * tp] = phi_neg[0:RQ]
            for ch in range(NCH):
                phik = jnp.concatenate([phi_pos[RQ + ch * CR:RQ + (ch + 1) * CR],
                                        phi_neg[RQ + ch * CR:RQ + (ch + 1) * CR]], axis=0)
                vta = jnp.concatenate([vT[ch * CV:(ch + 1) * CV], ones_pad], axis=0)
                kvz_acc[ch] += _dg(phik, vta, 1, 1)
        lhs_kv, lhs_z = [], []
        for ch in range(NCH):
            kvz = kvz_acc[ch]
            lhs_kv.append(jnp.where(bdmask2, kvz[:, 0:CV], 0.0).astype(jnp.bfloat16))
            zb = jnp.broadcast_to(kvz[:, CV:CV + 1], (2 * CR, CV))
            lhs_z.append(jnp.where(bdmask2, zb, 0.0).astype(jnp.bfloat16))
        for t in range(n_tiles):
            oTs = []
            for ch in range(NCH):
                phiq = jnp.concatenate([phiq_st[ch * CR:(ch + 1) * CR, t * tp:(t + 1) * tp],
                                        phiq_st[RQ + ch * CR:RQ + (ch + 1) * CR, t * tp:(t + 1) * tp]], axis=0)
                numT = _dg(lhs_kv[ch], phiq, 0, 0)
                denT = _dg(lhs_z[ch], phiq, 0, 0)
                oTs.append((numT * (1.0 / (denT + 1e-6))).astype(jnp.bfloat16))
            oT = jnp.concatenate(oTs, axis=0)
            x_vm[t * tp:(t + 1) * tp, :] = x_vm[t * tp:(t + 1) * tp, :] + _dg(oT, wo_ref[...], 0, 0)

    def layer_b():
        w1 = w1_ref[...]
        w2 = w2_ref[...]
        for t in range(n_tiles):
            xt = x_vm[t * tp:(t + 1) * tp, :]
            l = _layernorm(xt).astype(jnp.bfloat16)
            h = _dot(l, w1)
            h = h * jax.nn.sigmoid(h)
            x_vm[t * tp:(t + 1) * tp, :] = xt + _dot(h.astype(jnp.bfloat16), w2)

    layer_a()
    layer_b()
    layer_a()
    layer_b()
    o_ref[...] = x_vm[...].astype(o_ref.dtype)


@jax.jit
def pallas_interleave_layers__linear_kernel_hedgehog__dense_activation_silu__prompt_kernel(
    A_x: jax.Array,
    A_wqkv: jax.Array,
    A_w_phi: jax.Array,
    A_wo: jax.Array,
    B_x: jax.Array,
    B_w1: jax.Array,
    B_w2: jax.Array,
):
    del B_x
    tp = 256
    x = A_x.reshape(S, D)
    wpht = jnp.pad(A_w_phi.transpose(0, 2, 1), ((0, 0), (0, HP - DH), (0, 0))).reshape(RQ, DH)
    kern = functools.partial(_kernel, tp=tp)
    full = lambda shape: pl.BlockSpec(shape, lambda: (0,) * len(shape))
    out = pl.pallas_call(
        kern,
        out_shape=jax.ShapeDtypeStruct((S, D), A_x.dtype),
        in_specs=[full((S, D)), full((D, 3 * D)), full((RQ, DH)),
                  full((D, D)), full((D, F)), full((F, D))],
        out_specs=full((S, D)),
        scratch_shapes=[
            pltpu.VMEM((S, D), jnp.float32),
            pltpu.VMEM((2 * RQ, D), jnp.bfloat16),
            pltpu.VMEM((2 * RQ, S), jnp.bfloat16),
            pltpu.VMEM((NCH, 2 * CR, 128), jnp.float32),
        ],
        compiler_params=pltpu.CompilerParams(vmem_limit_bytes=100 * 1024 * 1024),
    )(x, A_wqkv, wpht, A_wo, B_w1, B_w2)
    return out.reshape(1, S, D)
```

```python
import functools

import jax
import jax.numpy as jnp
import jax.experimental.pallas as pl
import jax.experimental.pallas.tpu as pltpu

S, D, H, DH, F = 2048, 640, 32, 20, 1728
HP = 24
RQ = H * HP
NCH, HPC = 8, 4
CR = HPC * HP
CV = HPC * DH
EPS_LN = 1e-5
NEG = -1e30


def _layernorm(x):
    m = jnp.mean(x, axis=-1, keepdims=True)
    xc = x - m
    v = jnp.mean(xc * xc, axis=-1, keepdims=True)
    return xc * jax.lax.rsqrt(v + EPS_LN)


def _dot(a, b):
    return jnp.dot(a, b, preferred_element_type=jnp.float32)


def _dg(a, b, ca, cb):
    return jax.lax.dot_general(a, b, (((ca,), (cb,)), ((), ())), preferred_element_type=jnp.float32)


def _kernel(x_hbm, wqkv_hbm, wpht_ref, wo_hbm, w1t_hbm, w2_hbm, o_hbm,
            x_in, wqkv_ref, wo_ref, w1t_ref, w2_ref, x_vm, wqkt_vm, phiq_st, kvz_acc, oT_st,
            out_stage, sems, out_sems, *, tp):
    n_tiles = S // tp

    cp_x = pltpu.make_async_copy(x_hbm, x_in, sems.at[0])
    cp_wqkv = pltpu.make_async_copy(wqkv_hbm, wqkv_ref, sems.at[1])
    cp_wo = pltpu.make_async_copy(wo_hbm, wo_ref, sems.at[2])
    cp_w1 = pltpu.make_async_copy(w1t_hbm, w1t_ref, sems.at[3])
    cp_w2 = pltpu.make_async_copy(w2_hbm, w2_ref, sems.at[4])
    cp_wqkv.start()
    cp_x.start()
    cp_wo.start()
    cp_w1.start()
    cp_w2.start()
    cp_wqkv.wait()

    for h in range(H):
        wph = wpht_ref[h * HP:(h + 1) * HP, :]
        wq_h = wqkv_ref[:, h * DH:(h + 1) * DH]
        wk_h = wqkv_ref[:, D + h * DH:D + (h + 1) * DH]
        wqkt_vm[h * HP:(h + 1) * HP, :] = _dg(wph, wq_h, 1, 1).astype(jnp.bfloat16)
        wqkt_vm[RQ + h * HP:RQ + (h + 1) * HP, :] = _dg(wph, wk_h, 1, 1).astype(jnp.bfloat16)
    cp_x.wait()
    x_vm[...] = x_in[...].astype(jnp.float32)

    rowt = jax.lax.broadcasted_iota(jnp.int32, (2 * RQ, tp), 0)
    valid = (rowt % HP) < DH

    def softmax_branches(pT):
        outs = []
        for sgn in (1.0, -1.0):
            z = jnp.where(valid, sgn * pT, NEG).reshape(2 * H, HP, tp)
            m = jnp.max(z, axis=1, keepdims=True)
            e = jnp.exp(z - m)
            sm = jnp.sum(e, axis=1, keepdims=True)
            p = (e * (1.0 / sm)).reshape(2 * RQ, tp)
            outs.append(p.astype(jnp.bfloat16))
        return outs

    def layer_a(first):
        kvz_acc[...] = jnp.zeros_like(kvz_acc)
        wqkt = wqkt_vm[...]
        for t in range(n_tiles):
            xt = x_vm[t * tp:(t + 1) * tp, :]
            l = _layernorm(xt).astype(jnp.bfloat16)
            pT = _dg(wqkt, l, 1, 1)
            vT = _dg(wqkv_ref[:, 2 * D:3 * D], l, 0, 1).astype(jnp.bfloat16)
            phi_pos, phi_neg = softmax_branches(pT)
            phiq_st[0:RQ, t * tp:(t + 1) * tp] = phi_pos[0:RQ].astype(jnp.float32)
            phiq_st[RQ:2 * RQ, t * tp:(t + 1) * tp] = phi_neg[0:RQ].astype(jnp.float32)
            ones8 = jnp.ones((8, tp), jnp.bfloat16)
            for h in range(H):
                phik = jnp.concatenate([phi_pos[RQ + h * HP:RQ + (h + 1) * HP],
                                        phi_neg[RQ + h * HP:RQ + (h + 1) * HP]], axis=0)
                vaug = jnp.concatenate([vT[h * DH:(h + 1) * DH], ones8], axis=0)
                kvz_acc[h, 0:DH + 8, 0:2 * HP] += _dg(vaug, phik, 1, 1)
        if first:
            cp_wo.wait()
        kvz = [kvz_acc[h, 0:HP, 0:2 * HP].astype(jnp.bfloat16) for h in range(H)]
        for t in range(n_tiles):
            for h in range(H):
                phiq = jnp.concatenate([phiq_st[h * HP:(h + 1) * HP, t * tp:(t + 1) * tp],
                                        phiq_st[RQ + h * HP:RQ + (h + 1) * HP, t * tp:(t + 1) * tp]],
                                       axis=0).astype(jnp.bfloat16)
                nd = _dot(kvz[h], phiq)
                oth = nd[0:DH] * (1.0 / (nd[DH:DH + 1] + 1e-6))
                oT_st[h * DH:(h + 1) * DH, :] = oth.astype(jnp.bfloat16)
            x_vm[t * tp:(t + 1) * tp, :] = x_vm[t * tp:(t + 1) * tp, :] + _dg(oT_st[...], wo_ref[...], 0, 0)

    def layer_b(first, last):
        if first:
            cp_w1.wait()
            cp_w2.wait()
        w1t = w1t_ref[...]
        w2 = w2_ref[...]
        for t in range(n_tiles):
            xt = x_vm[t * tp:(t + 1) * tp, :]
            l = _layernorm(xt).astype(jnp.bfloat16)
            h = _dg(l, w1t, 1, 1)
            h = h * jax.nn.sigmoid(h)
            y = xt + _dot(h.astype(jnp.bfloat16), w2)
            x_vm[t * tp:(t + 1) * tp, :] = y
            if last:
                out_stage[t * tp:(t + 1) * tp, :] = y.astype(out_stage.dtype)
                pltpu.make_async_copy(out_stage.at[pl.ds(t * tp, tp), :],
                                      o_hbm.at[pl.ds(t * tp, tp), :], out_sems.at[t]).start()

    layer_a(True)
    layer_b(True, False)
    layer_a(False)
    layer_b(False, True)
    for t in range(n_tiles):
        pltpu.make_async_copy(out_stage.at[pl.ds(t * tp, tp), :],
                              o_hbm.at[pl.ds(t * tp, tp), :], out_sems.at[t]).wait()


@jax.jit
def pallas_interleave_layers__linear_kernel_hedgehog__dense_activation_silu__prompt_kernel(
    A_x: jax.Array,
    A_wqkv: jax.Array,
    A_w_phi: jax.Array,
    A_wo: jax.Array,
    B_x: jax.Array,
    B_w1: jax.Array,
    B_w2: jax.Array,
):
    del B_x
    tp = 256
    x = A_x.reshape(S, D)
    wpht = jnp.pad(A_w_phi.transpose(0, 2, 1), ((0, 0), (0, HP - DH), (0, 0))).reshape(RQ, DH)
    kern = functools.partial(_kernel, tp=tp)
    full = lambda shape: pl.BlockSpec(shape, lambda: (0,) * len(shape))
    hbm = pl.BlockSpec(memory_space=pl.ANY)
    out = pl.pallas_call(
        kern,
        out_shape=jax.ShapeDtypeStruct((S, D), A_x.dtype),
        in_specs=[hbm, hbm, full((RQ, DH)), hbm, hbm, hbm],
        out_specs=hbm,
        scratch_shapes=[
            pltpu.VMEM((S, D), A_x.dtype),
            pltpu.VMEM((D, 3 * D), A_wqkv.dtype),
            pltpu.VMEM((D, D), A_wo.dtype),
            pltpu.VMEM((F, D), B_w1.dtype),
            pltpu.VMEM((F, D), B_w2.dtype),
            pltpu.VMEM((S, D), jnp.float32),
            pltpu.VMEM((2 * RQ, D), jnp.bfloat16),
            pltpu.VMEM((2 * RQ, S), jnp.float32),
            pltpu.VMEM((H, 32, 128), jnp.float32),
            pltpu.VMEM((D, tp), jnp.bfloat16),
            pltpu.VMEM((S, D), A_x.dtype),
            pltpu.SemaphoreType.DMA((5,)),
            pltpu.SemaphoreType.DMA((S // tp,)),
        ],
        compiler_params=pltpu.CompilerParams(vmem_limit_bytes=100 * 1024 * 1024),
    )(x, A_wqkv, wpht, A_wo, B_w1.T, B_w2)
    return out.reshape(1, S, D)
```

```python
import functools

import jax
import jax.numpy as jnp
import jax.experimental.pallas as pl
import jax.experimental.pallas.tpu as pltpu

S, D, H, DH, F = 2048, 640, 32, 20, 1728
HP = 24
RQ = H * HP
NCH, HPC = 8, 4
CR = HPC * HP
CV = HPC * DH
EPS_LN = 1e-5
NEG = -1e30


def _layernorm(x):
    m = jnp.mean(x, axis=-1, keepdims=True)
    xc = x - m
    v = jnp.mean(xc * xc, axis=-1, keepdims=True)
    return xc * jax.lax.rsqrt(v + EPS_LN)


def _dot(a, b):
    return jnp.dot(a, b, preferred_element_type=jnp.float32)


def _dg(a, b, ca, cb):
    return jax.lax.dot_general(a, b, (((ca,), (cb,)), ((), ())), preferred_element_type=jnp.float32)


def _kernel(x_hbm, wqkv_hbm, wpht_ref, wo_hbm, w1t_hbm, w2_hbm, o_hbm,
            x_in, wqkv_ref, wo_ref, w1t_ref, w2_ref, x_vm, wqkt_vm, phiq_st, kvz_acc, oT_st,
            out_stage, sems, out_sems, *, tp):
    n_tiles = S // tp

    cp_x = pltpu.make_async_copy(x_hbm, x_in, sems.at[0])
    cp_wqkv = pltpu.make_async_copy(wqkv_hbm, wqkv_ref, sems.at[1])
    cp_wo = pltpu.make_async_copy(wo_hbm, wo_ref, sems.at[2])
    cp_w1 = pltpu.make_async_copy(w1t_hbm, w1t_ref, sems.at[3])
    cp_w2 = pltpu.make_async_copy(w2_hbm, w2_ref, sems.at[4])
    cp_wqkv.start()
    cp_x.start()
    cp_wo.start()
    cp_w1.start()
    cp_w2.start()
    cp_wqkv.wait()

    for h in range(H):
        wph = wpht_ref[h * HP:(h + 1) * HP, :]
        wq_h = wqkv_ref[:, h * DH:(h + 1) * DH]
        wk_h = wqkv_ref[:, D + h * DH:D + (h + 1) * DH]
        wqkt_vm[h * HP:(h + 1) * HP, :] = _dg(wph, wq_h, 1, 1).astype(jnp.bfloat16)
        wqkt_vm[RQ + h * HP:RQ + (h + 1) * HP, :] = _dg(wph, wk_h, 1, 1).astype(jnp.bfloat16)
    cp_x.wait()
    x_vm[...] = x_in[...].astype(jnp.float32)

    rowt = jax.lax.broadcasted_iota(jnp.int32, (2 * RQ, tp), 0)
    valid = (rowt % HP) < DH

    def softmax_branches(pT):
        outs = []
        for sgn in (1.0, -1.0):
            z = jnp.where(valid, sgn * pT, NEG).reshape(2 * H, HP, tp)
            m = jnp.max(z, axis=1, keepdims=True)
            e = jnp.exp(z - m)
            sm = jnp.sum(e, axis=1, keepdims=True)
            p = (e * (1.0 / sm)).reshape(2 * RQ, tp)
            outs.append(p.astype(jnp.bfloat16))
        return outs

    def layer_a(first):
        kvz_acc[...] = jnp.zeros_like(kvz_acc)
        wqkt = wqkt_vm[...]
        def project(t):
            xt = x_vm[t * tp:(t + 1) * tp, :]
            l = _layernorm(xt).astype(jnp.bfloat16)
            pT = _dg(wqkt, l, 1, 1)
            vT = _dg(wqkv_ref[:, 2 * D:3 * D], l, 0, 1).astype(jnp.bfloat16)
            return pT, vT
        ahead = [project(0), project(1)]
        for t in range(n_tiles):
            pT, vT = ahead.pop(0)
            if t + 2 < n_tiles:
                ahead.append(project(t + 2))
            phi_pos, phi_neg = softmax_branches(pT)
            phiq_st[0:RQ, t * tp:(t + 1) * tp] = phi_pos[0:RQ].astype(jnp.float32)
            phiq_st[RQ:2 * RQ, t * tp:(t + 1) * tp] = phi_neg[0:RQ].astype(jnp.float32)
            ones8 = jnp.ones((8, tp), jnp.bfloat16)
            for h in range(H):
                phik = jnp.concatenate([phi_pos[RQ + h * HP:RQ + (h + 1) * HP],
                                        phi_neg[RQ + h * HP:RQ + (h + 1) * HP]], axis=0)
                vaug = jnp.concatenate([vT[h * DH:(h + 1) * DH], ones8], axis=0)
                kvz_acc[h, 0:DH + 8, 0:2 * HP] += _dg(vaug, phik, 1, 1)
        if first:
            cp_wo.wait()
        kvz = [kvz_acc[h, 0:HP, 0:2 * HP].astype(jnp.bfloat16) for h in range(H)]
        for t in range(n_tiles):
            for h in range(H):
                phiq = jnp.concatenate([phiq_st[h * HP:(h + 1) * HP, t * tp:(t + 1) * tp],
                                        phiq_st[RQ + h * HP:RQ + (h + 1) * HP, t * tp:(t + 1) * tp]],
                                       axis=0).astype(jnp.bfloat16)
                nd = _dot(kvz[h], phiq)
                oth = nd[0:DH] * (1.0 / (nd[DH:DH + 1] + 1e-6))
                oT_st[h * DH:(h + 1) * DH, :] = oth.astype(jnp.bfloat16)
            x_vm[t * tp:(t + 1) * tp, :] = x_vm[t * tp:(t + 1) * tp, :] + _dg(oT_st[...], wo_ref[...], 0, 0)

    def layer_b(first, last):
        if first:
            cp_w1.wait()
            cp_w2.wait()
        w1t = w1t_ref[...]
        w2 = w2_ref[...]
        for t in range(n_tiles):
            xt = x_vm[t * tp:(t + 1) * tp, :]
            l = _layernorm(xt).astype(jnp.bfloat16)
            h = _dg(l, w1t, 1, 1)
            h = h * jax.nn.sigmoid(h)
            y = xt + _dot(h.astype(jnp.bfloat16), w2)
            x_vm[t * tp:(t + 1) * tp, :] = y
            if last:
                out_stage[t * tp:(t + 1) * tp, :] = y.astype(out_stage.dtype)
                pltpu.make_async_copy(out_stage.at[pl.ds(t * tp, tp), :],
                                      o_hbm.at[pl.ds(t * tp, tp), :], out_sems.at[t]).start()

    layer_a(True)
    layer_b(True, False)
    layer_a(False)
    layer_b(False, True)
    for t in range(n_tiles):
        pltpu.make_async_copy(out_stage.at[pl.ds(t * tp, tp), :],
                              o_hbm.at[pl.ds(t * tp, tp), :], out_sems.at[t]).wait()


@jax.jit
def pallas_interleave_layers__linear_kernel_hedgehog__dense_activation_silu__prompt_kernel(
    A_x: jax.Array,
    A_wqkv: jax.Array,
    A_w_phi: jax.Array,
    A_wo: jax.Array,
    B_x: jax.Array,
    B_w1: jax.Array,
    B_w2: jax.Array,
):
    del B_x
    tp = 256
    x = A_x.reshape(S, D)
    wpht = jnp.pad(A_w_phi.transpose(0, 2, 1), ((0, 0), (0, HP - DH), (0, 0))).reshape(RQ, DH)
    kern = functools.partial(_kernel, tp=tp)
    full = lambda shape: pl.BlockSpec(shape, lambda: (0,) * len(shape))
    hbm = pl.BlockSpec(memory_space=pl.ANY)
    out = pl.pallas_call(
        kern,
        out_shape=jax.ShapeDtypeStruct((S, D), A_x.dtype),
        in_specs=[hbm, hbm, full((RQ, DH)), hbm, hbm, hbm],
        out_specs=hbm,
        scratch_shapes=[
            pltpu.VMEM((S, D), A_x.dtype),
            pltpu.VMEM((D, 3 * D), A_wqkv.dtype),
            pltpu.VMEM((D, D), A_wo.dtype),
            pltpu.VMEM((F, D), B_w1.dtype),
            pltpu.VMEM((F, D), B_w2.dtype),
            pltpu.VMEM((S, D), jnp.float32),
            pltpu.VMEM((2 * RQ, D), jnp.bfloat16),
            pltpu.VMEM((2 * RQ, S), jnp.float32),
            pltpu.VMEM((H, 32, 128), jnp.float32),
            pltpu.VMEM((D, tp), jnp.bfloat16),
            pltpu.VMEM((S, D), A_x.dtype),
            pltpu.SemaphoreType.DMA((5,)),
            pltpu.SemaphoreType.DMA((S // tp,)),
        ],
        compiler_params=pltpu.CompilerParams(vmem_limit_bytes=100 * 1024 * 1024),
    )(x, A_wqkv, wpht, A_wo, B_w1.T, B_w2)
    return out.reshape(1, S, D)
```
